```python
import os as _os
_os.environ.setdefault("JAX_PLATFORMS", "cpu")
import jax
import jax.numpy as jnp

def _softmax(x, axis=-1):
    return jax.nn.softmax(x, axis=axis)
def _gelu(x):
    return jax.nn.gelu(x, approximate=True)
def _silu(x):
    return jax.nn.silu(x)
def _sigmoid(x):
    return jax.nn.sigmoid(x)
def _layernorm(x, axis=-1, eps=1e-5):
    m = jnp.mean(x, axis=axis, keepdims=True)
    v = jnp.var(x, axis=axis, keepdims=True)
    return (x - m) / jnp.sqrt(v + eps)
def _scatter_add(tgt, idx, src, axis=0):
    return tgt.at[idx].add(src)
def _segment_sum(src, seg, n):
    return jax.ops.segment_sum(src, seg, n)
class _Rng:
    def __init__(self, key):
        self._k = key
    def _next(self):
        self._k, sub = jax.random.split(self._k)
        return sub
    def normal(self, shape):
        return jax.random.normal(self._next(), shape, dtype=jnp.bfloat16)
    def randint(self, lo, hi, shape):
        return jax.random.randint(self._next(), shape, lo, hi, dtype=jnp.int32)
    def uniform(self, shape, lo=0.0, hi=1.0):
        return jax.random.uniform(self._next(), shape, jnp.bfloat16, lo, hi)
    def permutation(self, n):
        return jax.random.permutation(self._next(), n)


kernel_name = 'concat_heads__sliding_block_cached__compressed_kv_cla__decode'

def setup_inputs():
    _rng = _Rng(jax.random.key(int.from_bytes(__import__("os").urandom(4), "little")))
    _w = (lambda a: (lambda t: t.astype(jnp.bfloat16) if jnp.issubdtype(t.dtype, jnp.floating) else t)(jnp.asarray(a)))
    def _A_setup():
        B, Sq, D = 1, 1, 512
        Hq, Hkv, Sk, Dh = 32, 32, 4096, 128
        assert Hq % Hkv == 0, (Hq, Hkv)
        return {
            "x": _w((lambda *s: _rng.normal(s) * 0.8)(B, Sq, D)),
            "k_cache": _w((lambda *s: _rng.normal(s) * 0.8)(B, Hkv, Sk, Dh)),
            "v_cache": _w((lambda *s: _rng.normal(s) * 0.05)(B, Hkv, Sk, Dh)),
            "wq": _w((lambda *s: _rng.normal(s) * 0.8)(D, Hq * Dh) * (D ** -0.5)),
            "wo": _w((lambda *s: _rng.normal(s) * 0.05)(Hq * Dh, D) * ((Hq * Dh) ** -0.5)),
        }
    _A_in = _A_setup()

    def _B_setup():
        B, H, Sq, Sk, D, M = 1, 32, 1, 4096, 128, 512
        Dc = 4 * D
        return {
            "x": _w((lambda *s: _rng.normal(s) * 1.6)(B, Sq, M)),
            "c_kv": _w((lambda *s: _rng.normal(s) * 0.1)(B, Sk, Dc)),
            "w_q": _w((lambda *s: _rng.normal(s) * 1.6)(M, H, D) * (M ** -0.5)),
            "w_uk": _w((lambda *s: _rng.normal(s) * 1.6)(Dc, H, D) * (Dc ** -0.5)),
            "w_uv": _w((lambda *s: _rng.normal(s) * 0.1)(Dc, H, D) * (Dc ** -0.5)),
            "w_o": _w((lambda *s: _rng.normal(s) * 0.1)(H, D, M) * ((H * D) ** -0.5)),
        }
    _B_in = _B_setup()

    return {
        "A_x": _A_in["x"],
        "A_k_cache": _A_in["k_cache"],
        "A_v_cache": _A_in["v_cache"],
        "A_wq": _A_in["wq"],
        "A_wo": _A_in["wo"],
        "B_x": _B_in["x"],
        "B_c_kv": _B_in["c_kv"],
        "B_w_q": _B_in["w_q"],
        "B_w_uk": _B_in["w_uk"],
        "B_w_uv": _B_in["w_uv"],
        "B_w_o": _B_in["w_o"],
    }

def reference(A_x, A_k_cache, A_v_cache, A_wq, A_wo, B_x, B_c_kv, B_w_q, B_w_uk, B_w_uv, B_w_o):
    def _A_ref(x, k_cache, v_cache, wq, wo):
        B, Sq, D = x.shape
        Hq, Dh = 32, 128
        Hkv, Sk = k_cache.shape[1], k_cache.shape[2]
        W = min(4096, max(256, Sk // 4))
        rep = Hq // Hkv
        q = (lambda x, *d: x.transpose(*d))((x @ wq).reshape(B, Sq, Hq, Dh), 0, 2, 1, 3)
        k = jnp.repeat(k_cache[:, :, Sk - W:, :], rep, axis=1)
        v = jnp.repeat(v_cache[:, :, Sk - W:, :], rep, axis=1)
        scores = jnp.einsum("bhqd,bhkd->bhqk", q, k) * (Dh ** -0.5)
        p = _softmax(scores, axis=-1)
        o = jnp.einsum("bhqk,bhkd->bhqd", p, v)
        return (lambda x, *d: x.transpose(*d))(o, 0, 2, 1, 3).reshape(B, Sq, Hq * Dh) @ wo

    def _B_ref(x, c_kv, w_q, w_uk, w_uv, w_o):
        B, Sq, M = x.shape[0], x.shape[1], x.shape[2]
        Sk = c_kv.shape[1]
        H, D = w_q.shape[1], w_q.shape[2]
        q = jnp.einsum("bqm,mhd->bhqd", x, w_q)
        k = jnp.einsum("bkc,chd->bhkd", c_kv, w_uk)
        v = jnp.einsum("bkc,chd->bhkd", c_kv, w_uv)
        scores = jnp.einsum("bhqd,bhkd->bhqk", q, k) * (D ** -0.5)
        off = Sk - Sq
        qi = jnp.arange(Sq)[:, None]
        kj = jnp.arange(Sk)[None, :]
        cmask = kj <= (qi + off)
        scores = jnp.where(cmask[None, None], scores, -1e9)
        p = _softmax(scores, axis=-1)
        ctx = jnp.einsum("bhqk,bhkd->bhqd", p, v)
        return jnp.einsum("bhqd,hdm->bqm", ctx, w_o)

    a = _A_ref(A_x, A_k_cache, A_v_cache, A_wq, A_wo)
    b = _B_ref(B_x, B_c_kv, B_w_q, B_w_uk, B_w_uv, B_w_o)
    return jnp.concatenate([a, b], axis=-1)
```

```python
import jax
import jax.numpy as jnp
from jax import lax
from jax.experimental import pallas as pl
from jax.experimental.pallas import tpu as pltpu

BF = jnp.bfloat16
F32 = jnp.float32

H = 32
DH = 128
DM = 512
SK = 4096
WIN = 1024
DC = 512

NT = (((1,), (1,)), ((), ()))


def make(look=4, order=("bq", "uk", "c", "uv", "wq", "kv", "bo", "wo"), compute=True, **cp):
    def kernel(ax_h, k_h, v_h, wq_h, wo_h, bx_h, c_h, bq_h, uk_h, uv_h, bo_h, out_ref,
               ax_v, bx_v, k_v, v_v, wq_v, wo_v, c_v, bq_v, uk_v, uv_v, bo_v,
               r_s, qa_s, oa_s, ctx_s, xsem, sems):
        def slab(src, dst):
            def f(i):
                return [(src.at[pl.ds(2 * p, 2), pl.ds(i * 16, 16)],
                         dst.at[pl.ds(2 * p, 2), pl.ds(i * 16, 16)]) for p in range(2)]
            return f

        def rows(src, dst):
            def f(i):
                return [(src.at[pl.ds(i * 512 + p * 256, 256)],
                         dst.at[pl.ds(i * 512 + p * 256, 256)]) for p in range(2)]
            return f

        def wq_cp(i):
            return [(wq_h.at[pl.ds(p * 256, 256), pl.ds(i * 512, 512)],
                     wq_v.at[i, pl.ds(p * 256, 256)]) for p in range(2)]

        def kv_cp(i):
            return [(k_h.at[i, pl.ds(SK - WIN, WIN)], k_v.at[i]),
                    (v_h.at[i, pl.ds(SK - WIN, WIN)], v_v.at[i])]

        phases = dict(
            bq=(8, slab(bq_h, bq_v)), uk=(8, slab(uk_h, uk_v)), uv=(8, slab(uv_h, uv_v)),
            c=(8, rows(c_h, c_v)), wo=(8, rows(wo_h, wo_v)), bo=(8, rows(bo_h, bo_v)),
            wq=(8, wq_cp), kv=(32, kv_cp))
        base = {}
        tot = 0
        for name in order:
            base[name] = tot
            tot += phases[name][0]

        def copies(name, i):
            g = base[name] + i
            slot = g % look if isinstance(g, int) else lax.rem(g, look)
            return [pltpu.make_async_copy(s, d, sems.at[slot])
                    for p, (s, d) in enumerate(phases[name][1](i))]

        def start(name, i):
            for p, cp in enumerate(copies(name, i)):
                cp.start(priority=p)

        def advance(name, i):
            n = phases[name][0]
            for cp in copies(name, i):
                cp.wait()
            pos = order.index(name)

            @pl.when(i + look < n)
            def _():
                start(name, i + look)

            if pos + 1 < len(order):
                @pl.when(i + look >= n)
                def _():
                    start(order[pos + 1], i + look - n)

        x_cps = [pltpu.make_async_copy(bx_h, bx_v, xsem),
                 pltpu.make_async_copy(ax_h, ax_v, xsem)]
        start(order[0], 0)
        for cp in x_cps:
            cp.start()
        for i in range(1, look):
            start(order[0], i)
        for cp in x_cps:
            cp.wait()

        diag = (lax.broadcasted_iota(jnp.int32, (H, 128), 1) % H
                == lax.broadcasted_iota(jnp.int32, (H, 128), 0))

        def tile(w_v, t):
            return jnp.concatenate([w_v[i, t] for i in range(4)], axis=0)

        def head_contract(name, w_v):
            def body(i, acc):
                advance(name, i)
                if not compute:
                    return acc
                for u in range(16):
                    t = i * 16 + u
                    row = jnp.broadcast_to(r_s[pl.ds(t, 1), :], (H, 128))
                    lhs = jnp.where(diag, row, 0.0).astype(BF)
                    acc = acc + jnp.dot(lhs, tile(w_v, t), preferred_element_type=F32)
                return acc
            return lax.fori_loop(0, 8, body, jnp.zeros((H, 128), F32))

        def out_proj(name, src_s, w_v):
            def body(i, acc):
                advance(name, i)
                if not compute:
                    return acc
                lhs = jnp.concatenate(
                    [jnp.broadcast_to(src_s[pl.ds(i * 4 + u, 1), :], (8, DH)) for u in range(4)],
                    axis=1).astype(BF)
                w = w_v[pl.ds(pl.multiple_of(i * 512, 512), 512), :]
                return acc + jnp.dot(lhs, w, preferred_element_type=F32)
            return lax.fori_loop(0, 8, body, jnp.zeros((8, DM), F32))

        state = {}

        def run_bq():
            xb = bx_v[0].astype(F32)
            rt = jnp.concatenate(
                [jnp.broadcast_to(xb[:, i * 128:(i + 1) * 128], (H, 128)) for i in range(4)], axis=0)
            r_s[...] = rt.T
            state["qb"] = head_contract("bq", bq_v).astype(BF)

        def run_uk():
            qb = state["qb"]

            def body(i, carry):
                advance("uk", i)
                if not compute:
                    return carry
                for u in range(16):
                    t = i * 16 + u
                    o = lax.dot_general(qb, tile(uk_v, t), NT, preferred_element_type=F32)
                    r_s[pl.ds(t, 1), :] = jnp.sum(jnp.where(diag, o, 0.0), axis=0, keepdims=True)
                return carry
            lax.fori_loop(0, 8, body, 0)
            rt = r_s[...].T
            state["qabs"] = jnp.concatenate(
                [rt[i * H:(i + 1) * H, :] for i in range(4)], axis=1).astype(BF)

        def run_c():
            qabs = state["qabs"]

            def body(i, carry):
                m, l, acc = carry
                advance("c", i)
                if not compute:
                    return carry
                c = c_v[pl.ds(pl.multiple_of(i * 512, 512), 512), :]
                s = lax.dot_general(qabs, c, NT, preferred_element_type=F32) * (DH ** -0.5)
                m_new = jnp.maximum(m, jnp.max(s, axis=1, keepdims=True))
                alpha = jnp.exp(m - m_new)
                p = jnp.exp(s - m_new)
                l = alpha * l + jnp.sum(p, axis=1, keepdims=True)
                acc = alpha * acc + jnp.dot(p.astype(BF), c, preferred_element_type=F32)
                return m_new, l, acc
            m, l, acc = lax.fori_loop(
                0, 8, body,
                (jnp.full((H, 1), -jnp.inf, F32), jnp.zeros((H, 1), F32), jnp.zeros((H, DC), F32)))
            ctxc = acc / l
            rt = jnp.concatenate([ctxc[:, i * 128:(i + 1) * 128] for i in range(4)], axis=0)
            r_s[...] = rt.T

        def run_uv():
            ctx_s[...] = head_contract("uv", uv_v)

        def run_wq():
            xa = jnp.broadcast_to(ax_v[0].astype(F32), (8, DM)).astype(BF)

            def body(i, carry):
                advance("wq", i)
                if not compute:
                    return carry
                q = jnp.dot(xa, wq_v[i], preferred_element_type=F32)
                for u in range(4):
                    qa_s[i * 4 + u] = q[:, u * DH:(u + 1) * DH]
                return carry
            lax.fori_loop(0, 8, body, 0)

        def run_kv():
            def body(h, carry):
                advance("kv", h)
                if not compute:
                    return carry
                q = qa_s[h].astype(BF)
                s = lax.dot_general(q, k_v[h], NT, preferred_element_type=F32) * (DH ** -0.5)
                m = jnp.max(s, axis=1, keepdims=True)
                p = jnp.exp(s - m)
                l = jnp.sum(p, axis=1, keepdims=True)
                o = jnp.dot(p.astype(BF), v_v[h], preferred_element_type=F32) / l
                oa_s[pl.ds(h, 1), :] = o[0:1]
                return carry
            lax.fori_loop(0, H, body, 0)

        def run_bo():
            b = out_proj("bo", ctx_s, bo_v)
            out_ref[0, :, DM:2 * DM] = b[0:1].astype(out_ref.dtype)

        def run_wo():
            a = out_proj("wo", oa_s, wo_v)
            out_ref[0, :, 0:DM] = a[0:1].astype(out_ref.dtype)

        runs = dict(bq=run_bq, uk=run_uk, c=run_c, uv=run_uv, wq=run_wq, kv=run_kv, bo=run_bo, wo=run_wo)
        for name in order:
            runs[name]()

    def fn(A_x, A_k_cache, A_v_cache, A_wq, A_wo, B_x, B_c_kv, B_w_q, B_w_uk, B_w_uv, B_w_o):
        hbm = pl.BlockSpec(memory_space=pltpu.HBM)
        slab_shape = (4, DC // 4, H, DH)
        return pl.pallas_call(
            kernel,
            out_shape=jax.ShapeDtypeStruct((1, 1, 2 * DM), BF),
            in_specs=[hbm] * 11,
            out_specs=pl.BlockSpec(memory_space=pltpu.VMEM),
            scratch_shapes=[
                pltpu.VMEM((1, 1, DM), BF), pltpu.VMEM((1, 1, DM), BF),
                pltpu.VMEM((H, WIN, DH), BF), pltpu.VMEM((H, WIN, DH), BF),
                pltpu.VMEM((8, DM, 512), BF), pltpu.VMEM((H * DH, DM), BF),
                pltpu.VMEM((SK, DC), BF),
                pltpu.VMEM(slab_shape, BF), pltpu.VMEM(slab_shape, BF), pltpu.VMEM(slab_shape, BF),
                pltpu.VMEM((H * DH, DM), BF),
                pltpu.VMEM((128, 128), F32), pltpu.VMEM((H, 8, DH), F32),
                pltpu.VMEM((H, DH), F32), pltpu.VMEM((H, DH), F32),
                pltpu.SemaphoreType.DMA(()), pltpu.SemaphoreType.DMA((look,)),
            ],
            compiler_params=pltpu.CompilerParams(vmem_limit_bytes=100 * 2**20, **cp),
        )(A_x, A_k_cache.reshape(H, SK, DH), A_v_cache.reshape(H, SK, DH), A_wq, A_wo,
          B_x, B_c_kv.reshape(SK, DC), B_w_q.reshape(slab_shape), B_w_uk.reshape(slab_shape),
          B_w_uv.reshape(slab_shape), B_w_o.reshape(H * DH, DM))
    return fn


@jax.jit
def pallas_concat_heads__sliding_block_cached__compressed_kv_cla__decode_kernel(
    A_x, A_k_cache, A_v_cache, A_wq, A_wo, B_x, B_c_kv, B_w_q, B_w_uk, B_w_uv, B_w_o):
    return make()(A_x, A_k_cache, A_v_cache, A_wq, A_wo, B_x, B_c_kv, B_w_q, B_w_uk, B_w_uv, B_w_o)
```

```python
import jax
import jax.numpy as jnp
from jax import lax
from jax.experimental import pallas as pl
from jax.experimental.pallas import tpu as pltpu

BF16 = jnp.bfloat16
F32 = jnp.float32

H = 32
DH = 128
DM = 512
SK = 4096
WIN = min(4096, max(256, SK // 4))
DC = 512
SCALE = DH ** -0.5

STEPS = 8
LAG = 5
VPU_ROWS = 112
ORDER = ("bq", "uk", "c", "wq", "uv", "k0", "k1", "v0", "v1", "bo", "wo")

NT = (((1,), (1,)), ((), ()))


def _kernel(ax_h, k_h, v_h, wq_h, wo_h, bx_h, c_h, bq_h, uk_h, uv_h, bo_h, out_ref,
           ax_v, bx_v, k_v, v_v, wq_v, wo_v, c_v, bq_v, uk_v, uv_v, bo_v,
           r_s, sb_s, qa_s, sa_s, oa_s, ctx_s):

    def slabs(src, dst):
        def piece(i, u, cut):
            ix = (slice(None), u % 2, i * 8 + u // 2, cut(H))
            return src.at[ix], dst.at[ix]
        return piece, lambda i: dst.at[:, :, pl.ds(i * 8, 8)]

    def c_piece(i, u, cut):
        ix = (slice(None), u % 2, pl.ds(i * 64 + (u // 2) * 8, 8), cut(DC))
        return c_h.at[ix], c_v.at[ix]

    def wq_piece(i, u, cut):
        cols = cut(512)
        c0 = ((i // 4) * 4 + (u // 2) % 4) * 512
        ix = (slice(None), u % 2, pl.ds((i % 4) * 16 + (u // 8) * 8, 8),
              pl.ds(c0 + cols.start, cols.size))
        return wq_h.at[ix], wq_v.at[ix]

    def window(src, dst, h0):
        def piece(i, u, cut):
            keys = cut(32)
            heads = pl.ds(h0 + (i // 4) * 8 + (u % 2) * 4, 4)
            k0 = (i % 4) * 256 + (u // 2) * 32 + keys.start
            return (src.at[heads, pl.ds(SK - WIN + k0, keys.size)],
                    dst.at[heads, pl.ds(k0, keys.size)])
        return piece, lambda i: dst.at[pl.ds(h0 + (i // 4) * 8, 8), pl.ds((i % 4) * 256, 256)]

    def out_heads(src, dst, n=4):
        def piece(i, u, cut):
            ix = (pl.ds(0, n), pl.ds(i * DH + u * 8, 8), cut(DM))
            return src.at[ix], dst.at[ix]
        return piece, lambda i: dst.at[pl.ds(0, n), pl.ds(i * DH, DH)]

    phases = dict(
        bq=slabs(bq_h, bq_v), uk=slabs(uk_h, uk_v), uv=slabs(uv_h, uv_v),
        c=(c_piece, lambda i: c_v.at[:, :, pl.ds(i * 64, 64)]),
        wq=(wq_piece, lambda i: wq_v.at[:, :, pl.ds((i % 4) * 16, 16), pl.ds((i // 4) * 2048, 2048)]),
        k0=window(k_h, k_v, 0), k1=window(k_h, k_v, 16),
        v0=window(v_h, v_v, 0), v1=window(v_h, v_v, 16),
        bo=out_heads(bo_h, bo_v), wo=out_heads(wo_h, wo_v), wo_end=out_heads(wo_h, wo_v, 2))

    last = (STEPS - 1) * DH
    end_pieces = (((2, pl.ds(last, DH)), (3, pl.ds(last, DH - VPU_ROWS))),
                  ((3, pl.ds(last + DH - VPU_ROWS, VPU_ROWS)),))

    def end_copies(stage, sem):
        return [pltpu.make_async_copy(wo_h.at[ix], wo_v.at[ix], sem) for ix in end_pieces[stage]]

    def start(name, i, quarter, sem):
        piece, u0 = phases[name][0], 4 * quarter
        pltpu.make_async_copy(*piece(i, u0, lambda n: pl.ds(0, n // 4)), sem).start(priority=0)
        pltpu.make_async_copy(*piece(i, u0, lambda n: pl.ds(n // 4, n - n // 4)), sem).start(priority=1)
        for u in range(u0 + 1, u0 + 4):
            pltpu.make_async_copy(*piece(i, u, lambda n: pl.ds(0, n)), sem).start(priority=1)

    def wait(name, i, sem):
        buf = phases[name][1](i)
        pltpu.make_async_copy(buf, buf, sem).wait()

    diag = (lax.broadcasted_iota(jnp.int32, (H, 128), 1) % H
            == lax.broadcasted_iota(jnp.int32, (H, 128), 0))

    def head_row(src_s, h):
        return jnp.broadcast_to(src_s[pl.ds(h, 1), :], (8, src_s.shape[1])).astype(BF16)

    def project(src_s, w_v, i, group, n=DH):
        r0 = i * DH if isinstance(i, int) else pl.multiple_of(i * DH, DH)
        return jnp.dot(head_row(src_s, group * 8 + i)[:, :n], w_v[group, pl.ds(r0, n), :],
                       preferred_element_type=F32)

    def stream(sems, end_sems):
        def run_phase(name, work, init=None, ahead=1):
            nxt = ORDER[ORDER.index(name) + 1]

            def body(i, carry):
                if ahead == 1:
                    wait(name, i, sems.at[i])
                else:
                    @pl.when(i % ahead == 0)
                    def _():
                        for j in range(ahead):
                            wait(name, i + j, sems.at[i + j])
                for quarter in range(4):
                    start(nxt, i, quarter, sems.at[i])
                    carry = work(i, quarter, carry)
                return carry
            return lax.fori_loop(0, STEPS, body, init)

        x_copies = [pltpu.make_async_copy(bx_h, bx_v, end_sems[2]),
                    pltpu.make_async_copy(ax_h, ax_v, end_sems[2])]
        for copy in x_copies:
            copy.start()

        def start_first(i, carry):
            for quarter in range(4):
                start(ORDER[0], i, quarter, sems.at[i])
            return carry
        lax.fori_loop(0, STEPS, start_first, None)
        for copy in x_copies:
            copy.wait()

        def tiles(w_v, i, quarter):
            for u in range(4 * quarter, 4 * quarter + 4):
                s, j = u % 2, i * 8 + u // 2
                yield s * 64 + j, jnp.concatenate([w_v[g, s, j] for g in range(4)], axis=0)

        def contract_per_head(name, w_v):
            def work(i, quarter, acc):
                for t, tile in tiles(w_v, i, quarter):
                    coef = jnp.broadcast_to(r_s[pl.ds(t, 1), :], (H, 128))
                    lhs = jnp.where(diag, coef, 0.0).astype(BF16)
                    acc = acc + jnp.dot(lhs, tile, preferred_element_type=F32)
                return acc
            return run_phase(name, work, jnp.zeros((H, DH), F32))

        xb = bx_v[0].astype(F32)
        r_s[...] = jnp.concatenate(
            [jnp.broadcast_to(xb[:, g * 128:(g + 1) * 128], (H, 128)) for g in range(4)], axis=0).T
        qb = contract_per_head("bq", bq_v).astype(BF16)

        def uk_work(i, quarter, carry):
            for t, tile in tiles(uk_v, i, quarter):
                o = lax.dot_general(qb, tile, NT, preferred_element_type=F32)
                r_s[pl.ds(t, 1), :] = jnp.sum(jnp.where(diag, o, 0.0), axis=0, keepdims=True)
            return carry
        run_phase("uk", uk_work)
        rt = r_s[...].T
        q_abs = jnp.concatenate([rt[g * H:(g + 1) * H, :] for g in range(4)], axis=1).astype(BF16)

        def c_block(i, quarter):
            keys = pl.ds(pl.multiple_of(i * 64, 64), 64)
            return jnp.concatenate([c_v[quarter, s, keys, :] for s in range(2)], axis=0)

        def c_work(i, quarter, m):
            s = lax.dot_general(q_abs, c_block(i, quarter), NT, preferred_element_type=F32) * SCALE
            sb_s[i * 4 + quarter] = s
            return jnp.maximum(m, s)
        mb = run_phase("c", c_work, jnp.full((H, 128), -jnp.inf, F32))
        mb = jnp.broadcast_to(jnp.max(mb, axis=1, keepdims=True), (H, 128))

        xa = jnp.broadcast_to(ax_v[0].astype(F32), (8, DM)).astype(BF16)

        def wq_work(i, quarter, carry):
            total, acc = carry
            cols = pl.ds(pl.multiple_of((i * 4 + quarter) * DH, DH), DH)
            w = jnp.concatenate([wq_v[g, s, :, cols] for g in range(4) for s in range(2)], axis=0)
            qa_s[i * 4 + quarter] = jnp.dot(xa, w, preferred_element_type=F32)
            p = jnp.exp(sb_s[i * 4 + quarter] - mb)
            acc = acc + jnp.dot(p.astype(BF16), c_block(i, quarter), preferred_element_type=F32)
            return total + p, acc
        total, acc = run_phase(
            "wq", wq_work, (jnp.zeros((H, 128), F32), jnp.zeros((H, DC), F32)), ahead=4)
        ctx_c = acc / jnp.sum(total, axis=1, keepdims=True)

        r_s[...] = jnp.concatenate(
            [ctx_c[:, g * 128:(g + 1) * 128] for g in range(4)], axis=0).T
        ctx_s[...] = contract_per_head("uv", uv_v)

        def heads_and_keys(w_v, h0, i, quarter):
            keys = pl.ds(pl.multiple_of((i % 4) * 256, 256), 256)
            for j in range(2):
                h = h0 + (i // 4) * 8 + 2 * quarter + j
                yield h, w_v[h, keys, :]

        def k_work(h0):
            def work(i, quarter, carry):
                for h, k in heads_and_keys(k_v, h0, i, quarter):
                    s = lax.dot_general(qa_s[h].astype(BF16), k, NT, preferred_element_type=F32)
                    sa_s[i % 4, pl.ds(h, 1), :] = s[0:1] * SCALE
                return carry
            return work

        def v_work(h0):
            def work(i, quarter, carry):
                for h, v in heads_and_keys(v_v, h0, i, quarter):
                    o = jnp.dot(head_row(sa_s.at[i % 4], h), v, preferred_element_type=F32)
                    oa_s[pl.ds(h, 1), :] += o[0:1]
                return carry
            return work

        run_phase("k0", k_work(0))
        run_phase("k1", k_work(16))
        sa = [sa_s[j] for j in range(4)]
        ma = jnp.max(jnp.maximum(jnp.maximum(sa[0], sa[1]), jnp.maximum(sa[2], sa[3])),
                     axis=1, keepdims=True)
        pa = [jnp.exp(s - ma) for s in sa]
        inv = 1.0 / jnp.sum((pa[0] + pa[1]) + (pa[2] + pa[3]), axis=1, keepdims=True)
        for j in range(4):
            sa_s[j] = pa[j] * inv
        oa_s[...] = jnp.zeros((H, DH), F32)
        run_phase("v0", v_work(0))
        run_phase("v1", v_work(16))

        def out_step(i, carry, nxt, sem, follow):
            a, b = carry
            wait("bo", i, sems.at[i])
            if follow:
                wait("wo", i - LAG, sems.at[i - LAG])
            for quarter in range(4):
                start(nxt, i, quarter, sem)
                b = b + project(ctx_s, bo_v, i, quarter)
                if follow:
                    a = a + project(oa_s, wo_v, i - LAG, quarter)
            return a, b

        o_last = oa_s[pl.ds(H - 1, 1), :].astype(BF16).astype(F32)
        r_s[...] = jnp.broadcast_to(o_last, (DH, DH)).T
        zero = jnp.zeros((8, DM), F32)
        carry = lax.fori_loop(
            0, LAG, lambda i, c: out_step(i, c, "wo", sems.at[i], False), (zero, zero))
        carry = lax.fori_loop(
            LAG, STEPS - 1, lambda i, c: out_step(i, c, "wo", sems.at[i], True), carry)
        a, b = out_step(STEPS - 1, carry, "wo_end", end_sems[0], True)
        for stage in range(2):
            for copy in end_copies(stage, end_sems[1 + stage]):
                copy.start(priority=1)

        def wo_step(i, a):
            wait("wo", i, sems.at[i])
            for group in range(4):
                a = a + project(oa_s, wo_v, i, group)
            return a
        return lax.fori_loop(STEPS - LAG, STEPS - 1, wo_step, a), b

    dma_sem = pltpu.SemaphoreType.DMA

    def stage0(end_sems):
        a, b = pl.run_scoped(lambda sems: stream(sems, end_sems), dma_sem((STEPS,)))
        wait("wo_end", STEPS - 1, end_sems[0])
        return a, b

    def stage1(end_sems):
        a, b = pl.run_scoped(lambda sem: stage0([sem] + end_sems), dma_sem(()))
        a = a + project(oa_s, wo_v, STEPS - 1, 0) + project(oa_s, wo_v, STEPS - 1, 1)
        for copy in end_copies(0, end_sems[0]):
            copy.wait()
        return a, b

    def stage2(sem):
        a, b = pl.run_scoped(lambda sem1: stage1([sem1, sem]), dma_sem(()))
        a = a + project(oa_s, wo_v, STEPS - 1, 2) + project(oa_s, wo_v, STEPS - 1, 3, DH - VPU_ROWS)
        for copy in end_copies(1, sem):
            copy.wait()
        return a, b

    a, b = pl.run_scoped(stage2, dma_sem(()))
    coef = r_s[pl.ds(DH - VPU_ROWS, VPU_ROWS), :]
    rest = [jnp.sum(wo_v[3, pl.ds(last + DH - VPU_ROWS, VPU_ROWS), pl.ds(j * 128, 128)].astype(F32)
                    * coef, axis=0, keepdims=True) for j in range(DM // 128)]
    a = a[0:1] + jnp.concatenate(rest, axis=1)
    out_ref[0] = jnp.concatenate([a, b[0:1]], axis=1).astype(out_ref.dtype)


@jax.jit
def pallas_concat_heads__sliding_block_cached__compressed_kv_cla__decode_kernel(
    A_x: jax.Array,
    A_k_cache: jax.Array,
    A_v_cache: jax.Array,
    A_wq: jax.Array,
    A_wo: jax.Array,
    B_x: jax.Array,
    B_c_kv: jax.Array,
    B_w_q: jax.Array,
    B_w_uk: jax.Array,
    B_w_uv: jax.Array,
    B_w_o: jax.Array,
):
    slab = (4, 2, 64, H, DH)
    wq_shape = (4, 2, 64, H * DH)
    c_shape = (4, 2, SK // 8, DC)
    wo_shape = (4, 8 * DH, DM)
    return pl.pallas_call(
        _kernel,
        out_shape=jax.ShapeDtypeStruct((1, 1, 2 * DM), A_x.dtype),
        in_specs=[pl.BlockSpec(memory_space=pltpu.HBM)] * 11,
        out_specs=pl.BlockSpec(memory_space=pltpu.VMEM),
        scratch_shapes=[
            pltpu.VMEM((1, 1, DM), BF16), pltpu.VMEM((1, 1, DM), BF16),
            pltpu.VMEM((H, WIN, DH), BF16), pltpu.VMEM((H, WIN, DH), BF16),
            pltpu.VMEM(wq_shape, BF16), pltpu.VMEM(wo_shape, BF16), pltpu.VMEM(c_shape, BF16),
            pltpu.VMEM(slab, BF16), pltpu.VMEM(slab, BF16), pltpu.VMEM(slab, BF16),
            pltpu.VMEM(wo_shape, BF16),
            pltpu.VMEM((128, 128), F32), pltpu.VMEM((SK // 128, H, 128), F32),
            pltpu.VMEM((H, 8, DH), F32), pltpu.VMEM((4, H, WIN // 4), F32),
            pltpu.VMEM((H, DH), F32), pltpu.VMEM((H, DH), F32),
        ],
        compiler_params=pltpu.CompilerParams(vmem_limit_bytes=64 * 2**20),
    )(A_x, A_k_cache.reshape(H, SK, DH), A_v_cache.reshape(H, SK, DH),
      A_wq.reshape(wq_shape), A_wo.reshape(wo_shape),
      B_x, B_c_kv.reshape(c_shape), B_w_q.reshape(slab), B_w_uk.reshape(slab),
      B_w_uv.reshape(slab), B_w_o.reshape(wo_shape))
```

```python
import jax
import jax.numpy as jnp
from jax import lax
from jax.experimental import pallas as pl
from jax.experimental.pallas import tpu as pltpu

BF16 = jnp.bfloat16
F32 = jnp.float32

H = 32
DH = 128
DM = 512
SK = 4096
WIN = min(4096, max(256, SK // 4))
DC = 512
SCALE = DH ** -0.5

VPU_ROWS = 112

NT = (((1,), (1,)), ((), ()))


def _kernel(ax_h, k_h, v_h, wq_h, wo_h, bx_h, c_h, bq_h, uk_h, uv_h, bo_h, out_ref,
            ax_v, bx_v, k_v, v_v, wq_v, wo_v, c_v, bq_v, uk_v, uv_v, bo_v,
            r_s, sb_s, qa_s, sa_s, oa_s, ctx_s):

    def rows(src, dst, sem, g, j, n):
        def at(lo, size):
            ix = (g, pl.ds(j * n + lo, size))
            return pltpu.make_async_copy(src.at[ix], dst.at[ix], sem)
        return n, at

    def wq_rows(sem, g, j):
        def at(lo, size):
            ix = (g, pl.ds((j // 2) * 8, 8), pl.ds((j % 2) * 2048 + lo, size))
            return pltpu.make_async_copy(wq_h.at[ix], wq_v.at[ix], sem)
        return 2048, at

    def weights_step(sems, i):
        return [piece for g in range(4) for piece in (
            rows(bq_h, bq_v, sems.at[0], g, i, 128), wq_rows(sems.at[1], g, i),
            rows(uk_h, uk_v, sems.at[2], g, i, 128), rows(c_h, c_v, sems.at[3], g, i, 32),
            rows(uv_h, uv_v, sems.at[4], g, i, 128), rows(bo_h, bo_v, sems.at[5], g, i, 32))]

    def window_step(src, dst, sem, i):
        def piece(h):
            def at(lo, size):
                k0 = (i // 2) * 128 + lo
                return pltpu.make_async_copy(
                    src.at[h, pl.ds(SK - WIN + k0, size)], dst.at[h, pl.ds(k0, size)], sem)
            return 128, at
        return [piece((i % 2) * 16 + u) for u in range(16)]

    def wo_rows(sem, j0, n, groups=4):
        return [rows(wo_h, wo_v, sem, g, j0 + j, 32) for j in range(n) for g in range(groups)]

    def start(pieces):
        for u, (n, at) in enumerate(pieces):
            if u % 2:
                at(0, n).start(priority=1)
            else:
                at(0, n // 4).start(priority=0)
                at(n // 4, n - n // 4).start(priority=1)

    def wait(buf, sem):
        pltpu.make_async_copy(buf, buf, sem).wait()

    last = 7 * DH
    end_pieces = (((2, pl.ds(last, DH)), (3, pl.ds(last, DH - VPU_ROWS))),
                  ((3, pl.ds(last + DH - VPU_ROWS, VPU_ROWS)),))

    def end_copies(stage, sem):
        return [pltpu.make_async_copy(wo_h.at[ix], wo_v.at[ix], sem) for ix in end_pieces[stage]]

    dma_sem = pltpu.SemaphoreType.DMA

    diag = (lax.broadcasted_iota(jnp.int32, (H, 128), 1) % H
            == lax.broadcasted_iota(jnp.int32, (H, 128), 0))

    def head_row(src_s, h):
        return jnp.broadcast_to(src_s[pl.ds(h, 1), :], (8, src_s.shape[1])).astype(BF16)

    def project(src_s, w_v, i, group, n=DH):
        r0 = i * DH if isinstance(i, int) else pl.multiple_of(i * DH, DH)
        return jnp.dot(head_row(src_s, group * 8 + i)[:, :n], w_v[group, pl.ds(r0, n), :],
                       preferred_element_type=F32)

    def interleave(pieces, work, i, carry):
        n = len(pieces) // 4
        for quarter in range(4):
            start(pieces[n * quarter:n * (quarter + 1)])
            carry = work(i, quarter, carry)
        return carry

    def overlap(step, work, carry=None):
        return lax.fori_loop(0, 4, lambda i, c: interleave(step(i), work, i, c), carry)

    def tiles(w_v, i, quarter):
        for u in range(8):
            t = i * 32 + quarter * 8 + u
            yield t, jnp.concatenate(
                [w_v[g, pl.ds(pl.multiple_of(t * H, H), H), :] for g in range(4)], axis=0)

    def contract_per_head(w_v, i, quarter, acc):
        for t, tile in tiles(w_v, i, quarter):
            coef = jnp.broadcast_to(r_s[pl.ds(t, 1), :], (H, 128))
            lhs = jnp.where(diag, coef, 0.0).astype(BF16)
            acc = acc + jnp.dot(lhs, tile, preferred_element_type=F32)
        return acc

    def stream(sems, wo_sems, end_sems):
        k_sem, v_sem, wo_sem = sems.at[0], sems.at[1], sems.at[2]

        def k_step(i0):
            return lambda i: window_step(k_h, k_v, k_sem, i0 + i)

        def v_step(i0):
            return lambda i: window_step(v_h, v_v, v_sem, i0 + i)

        def v_wo_step(i0):
            def step(i):
                v = window_step(v_h, v_v, sems.at[3 + (i0 + i) // 2], 8 + i0 + i)
                wo = wo_rows(wo_sem, 2 * (i0 + i), 2)
                return [p for u in range(8) for p in (v[2 * u], v[2 * u + 1], wo[u])]
            return step

        def load_weights(weight_sems):
            x_copies = [pltpu.make_async_copy(bx_h, bx_v, weight_sems.at[6]),
                        pltpu.make_async_copy(ax_h, ax_v, weight_sems.at[7])]
            for copy in x_copies:
                copy.start()

            @pl.loop(0, 32)
            def _(i):
                start(weights_step(weight_sems, i))

            @pl.loop(0, 4)
            def _(i):
                start(k_step(0)(i))

            for copy in x_copies:
                copy.wait()
            for j, buf in enumerate((bq_v, wq_v, uk_v, c_v, uv_v, bo_v)):
                wait(buf, weight_sems.at[j])
        pl.run_scoped(load_weights, dma_sem((8,)))

        xb = bx_v[0].astype(F32)
        r_s[...] = jnp.concatenate(
            [jnp.broadcast_to(xb[:, g * 128:(g + 1) * 128], (H, 128)) for g in range(4)], axis=0).T
        xa = jnp.broadcast_to(ax_v[0].astype(F32), (8, DM)).astype(BF16)

        def q_work(i, quarter, acc):
            h = i * 8 + quarter * 2
            cols = pl.ds(pl.multiple_of(h * DH, 2 * DH), 2 * DH)
            w = jnp.concatenate([wq_v[g, :, cols] for g in range(4)], axis=0)
            qa = jnp.dot(xa, w, preferred_element_type=F32)
            qa_s[h] = qa[:, :DH]
            qa_s[h + 1] = qa[:, DH:]
            return contract_per_head(bq_v, i, quarter, acc)
        qb = overlap(k_step(4), q_work, jnp.zeros((H, DH), F32)).astype(BF16)

        def uk_work(i, quarter, carry):
            for t, tile in tiles(uk_v, i, quarter):
                o = lax.dot_general(qb, tile, NT, preferred_element_type=F32)
                r_s[pl.ds(t, 1), :] = jnp.sum(jnp.where(diag, o, 0.0), axis=0, keepdims=True)
            return carry
        overlap(k_step(8), uk_work)
        rt = r_s[...].T
        q_abs = jnp.concatenate([rt[g * H:(g + 1) * H, :] for g in range(4)], axis=1).astype(BF16)

        def c_block(i, quarter):
            return c_v[quarter, pl.ds(pl.multiple_of(i * 256, 256), 256), :]

        def score_work(i, quarter, m):
            s = lax.dot_general(q_abs, c_block(i, quarter), NT, preferred_element_type=F32) * SCALE
            sb_s[i * 4 + quarter] = s
            return jnp.maximum(m, s)
        mb = overlap(k_step(12), score_work, jnp.full((H, 256), -jnp.inf, F32))
        mb = jnp.broadcast_to(jnp.max(mb, axis=1, keepdims=True), (H, 256))

        def latent_work(i, quarter, carry):
            total, acc = carry
            p = jnp.exp(sb_s[i * 4 + quarter] - mb)
            return total + p, acc + jnp.dot(p.astype(BF16), c_block(i, quarter),
                                            preferred_element_type=F32)
        total, acc = overlap(v_step(0), latent_work,
                             (jnp.zeros((H, 256), F32), jnp.zeros((H, DC), F32)))
        ctx_c = acc / jnp.sum(total, axis=1, keepdims=True)
        r_s[...] = jnp.concatenate(
            [ctx_c[:, g * 128:(g + 1) * 128] for g in range(4)], axis=0).T

        def scores(h):
            s = lax.dot_general(qa_s[h].astype(BF16), k_v[h], NT, preferred_element_type=F32)
            for j in range(8):
                sa_s[j, pl.ds(h, 1), :] = s[0:1, j * 128:(j + 1) * 128] * SCALE

        def k0_work(i, quarter, acc):
            scores(i * 4 + quarter)
            return contract_per_head(uv_v, i, quarter, acc)
        wait(k_v, k_sem)
        ctx_s[...] = overlap(v_step(4), k0_work, jnp.zeros((H, DH), F32))
        overlap(v_wo_step(0), lambda i, quarter, carry: scores(16 + i * 4 + quarter))

        sa = sa_s[...]
        pa = jnp.exp(sa - jnp.max(jnp.max(sa, axis=0), axis=1, keepdims=True))
        sa_s[...] = pa / jnp.sum(jnp.sum(pa, axis=0), axis=1, keepdims=True)
        oa_s[...] = jnp.zeros((H, DH), F32)

        def values(j, quarter):
            for h in range(quarter * 8, quarter * 8 + 8):
                v = v_v[h, pl.ds(pl.multiple_of(j * 128, 128), 128), :]
                o = jnp.dot(head_row(sa_s.at[j], h), v, preferred_element_type=F32)
                oa_s[pl.ds(h, 1), :] += o[0:1]

        def v0_work(i, quarter, b):
            values(i, quarter)
            return b + project(ctx_s, bo_v, 2 * i, quarter) + project(ctx_s, bo_v, 2 * i + 1, quarter)
        wait(v_v.at[:, pl.ds(0, WIN // 2)], v_sem)
        b = overlap(v_wo_step(4), v0_work, jnp.zeros((8, DM), F32))

        def v1_round(i, pieces):
            wait(v_v.at[:, pl.ds((4 + i) * 128, 128)], sems.at[3 + i])
            interleave(pieces, lambda i, quarter, carry: values(4 + i, quarter), i, None)

        @pl.loop(0, 3)
        def _(i):
            v1_round(i, wo_rows(wo_sems.at[i], 4 * (4 + i), 4))
        v1_round(3, wo_rows(end_sems[0], 4 * 7, 4, groups=2))
        for stage in range(2):
            for copy in end_copies(stage, end_sems[1 + stage]):
                copy.start(priority=1)
        wait(wo_v.at[:, pl.ds(0, 4 * DH)], wo_sem)
        return b

    def finish(wo_sems, end_sems):
        b = pl.run_scoped(lambda sems: stream(sems, wo_sems, end_sems), dma_sem((7,)))
        o_last = oa_s[pl.ds(H - 1, 1), :].astype(BF16).astype(F32)
        r_s[...] = jnp.broadcast_to(o_last, (DH, DH)).T

        def heads(i, a):
            for group in range(4):
                a = a + project(oa_s, wo_v, i, group)
            return a

        def late_heads(i, a):
            wait(wo_v.at[:, pl.ds(i * DH, DH)], wo_sems.at[i - 4])
            return heads(i, a)
        a = lax.fori_loop(0, 4, heads, jnp.zeros((8, DM), F32), unroll=2)
        return lax.fori_loop(4, 7, late_heads, a), b

    def stage0(end_sems):
        a, b = pl.run_scoped(lambda sems: finish(sems, end_sems), dma_sem((3,)))
        wait(wo_v.at[pl.ds(0, 2), pl.ds(last, DH)], end_sems[0])
        return a, b

    def stage1(end_sems):
        a, b = pl.run_scoped(lambda sem: stage0([sem] + end_sems), dma_sem(()))
        a = a + project(oa_s, wo_v, 7, 0) + project(oa_s, wo_v, 7, 1)
        for copy in end_copies(0, end_sems[0]):
            copy.wait()
        return a, b

    def stage2(sem):
        a, b = pl.run_scoped(lambda sem1: stage1([sem1, sem]), dma_sem(()))
        a = a + project(oa_s, wo_v, 7, 2) + project(oa_s, wo_v, 7, 3, DH - VPU_ROWS)
        for copy in end_copies(1, sem):
            copy.wait()
        return a, b

    a, b = pl.run_scoped(stage2, dma_sem(()))
    coef = r_s[pl.ds(DH - VPU_ROWS, VPU_ROWS), :]
    rest = [jnp.sum(wo_v[3, pl.ds(last + DH - VPU_ROWS, VPU_ROWS), pl.ds(j * 128, 128)].astype(F32)
                    * coef, axis=0, keepdims=True) for j in range(DM // 128)]
    a = a[0:1] + jnp.concatenate(rest, axis=1)
    out_ref[0] = jnp.concatenate([a, b[0:1]], axis=1).astype(out_ref.dtype)


@jax.jit
def pallas_concat_heads__sliding_block_cached__compressed_kv_cla__decode_kernel(
    A_x: jax.Array,
    A_k_cache: jax.Array,
    A_v_cache: jax.Array,
    A_wq: jax.Array,
    A_wo: jax.Array,
    B_x: jax.Array,
    B_c_kv: jax.Array,
    B_w_q: jax.Array,
    B_w_uk: jax.Array,
    B_w_uv: jax.Array,
    B_w_o: jax.Array,
):
    slab = (4, 128 * H, DH)
    wide = (4, 128, H * DH)
    tall = (4, 1024, 512)
    return pl.pallas_call(
        _kernel,
        out_shape=jax.ShapeDtypeStruct((1, 1, 2 * DM), A_x.dtype),
        in_specs=[pl.BlockSpec(memory_space=pltpu.HBM)] * 11,
        out_specs=pl.BlockSpec(memory_space=pltpu.VMEM),
        scratch_shapes=[
            pltpu.VMEM((1, 1, DM), BF16), pltpu.VMEM((1, 1, DM), BF16),
            pltpu.VMEM((H, WIN, DH), BF16), pltpu.VMEM((H, WIN, DH), BF16),
            pltpu.VMEM(wide, BF16), pltpu.VMEM(tall, BF16), pltpu.VMEM(tall, BF16),
            pltpu.VMEM(slab, BF16), pltpu.VMEM(slab, BF16), pltpu.VMEM(slab, BF16),
            pltpu.VMEM(tall, BF16),
            pltpu.VMEM((128, 128), F32), pltpu.VMEM((SK // 256, H, 256), F32),
            pltpu.VMEM((H, 8, DH), F32), pltpu.VMEM((WIN // 128, H, 128), F32),
            pltpu.VMEM((H, DH), F32), pltpu.VMEM((H, DH), F32),
        ],
        compiler_params=pltpu.CompilerParams(vmem_limit_bytes=64 * 2**20),
    )(A_x, A_k_cache.reshape(H, SK, DH), A_v_cache.reshape(H, SK, DH),
      A_wq.reshape(wide), A_wo.reshape(tall),
      B_x, B_c_kv.reshape(tall), B_w_q.reshape(slab), B_w_uk.reshape(slab),
      B_w_uv.reshape(slab), B_w_o.reshape(tall))
```
